```python
import os as _os
_os.environ.setdefault("JAX_PLATFORMS", "cpu")
import jax
import jax.numpy as jnp

def _softmax(x, axis=-1):
    return jax.nn.softmax(x, axis=axis)
def _gelu(x):
    return jax.nn.gelu(x, approximate=True)
def _silu(x):
    return jax.nn.silu(x)
def _sigmoid(x):
    return jax.nn.sigmoid(x)
def _layernorm(x, axis=-1, eps=1e-5):
    m = jnp.mean(x, axis=axis, keepdims=True)
    v = jnp.var(x, axis=axis, keepdims=True)
    return (x - m) / jnp.sqrt(v + eps)
def _scatter_add(tgt, idx, src, axis=0):
    return tgt.at[idx].add(src)
def _segment_sum(src, seg, n):
    return jax.ops.segment_sum(src, seg, n)
class _Rng:
    def __init__(self, key):
        self._k = key
    def _next(self):
        self._k, sub = jax.random.split(self._k)
        return sub
    def normal(self, shape):
        return jax.random.normal(self._next(), shape, dtype=jnp.bfloat16)
    def randint(self, lo, hi, shape):
        return jax.random.randint(self._next(), shape, lo, hi, dtype=jnp.int32)
    def uniform(self, shape, lo=0.0, hi=1.0):
        return jax.random.uniform(self._next(), shape, jnp.bfloat16, lo, hi)
    def permutation(self, n):
        return jax.random.permutation(self._next(), n)


kernel_name = 'sequential_preLN__linear_attn_block__dense_activation_squared_relu__prompt'

def setup_inputs():
    _rng = _Rng(jax.random.key(int.from_bytes(__import__("os").urandom(4), "little")))
    _w = (lambda a: (lambda t: t.astype(jnp.bfloat16) if jnp.issubdtype(t.dtype, jnp.floating) else t)(jnp.asarray(a)))
    def _A_setup():
        B, S, D = 1, 2048, 576
        return {
            "x": _w((lambda *s: _rng.normal(s) * 0.05)(B, S, D)),
            "wqkv": _w((lambda *s: _rng.normal(s) * 0.1)(D, 3 * D)),
            "wo": _w((lambda *s: _rng.normal(s) * 0.05)(D, D)),
        }
    _A_in = _A_setup()

    def _B_setup():
        B, S, D, F = 1, 2048, 576, 4608
        return {
            "x": _w((lambda *s: _rng.normal(s) * 0.05)(B, S, D)),
            "w1": _w((lambda *s: _rng.normal(s) * 0.05)(D, F)),
            "b1": _w((lambda *s: _rng.normal(s) * 0.05)(F)),
            "w2": _w((lambda *s: _rng.normal(s) * 0.05)(F, D)),
            "b2": _w((lambda *s: _rng.normal(s) * 0.05)(D)),
        }
    _B_in = _B_setup()

    return {
        "A_x": _A_in["x"],
        "A_wqkv": _A_in["wqkv"],
        "A_wo": _A_in["wo"],
        "B_x": _B_in["x"],
        "B_w1": _B_in["w1"],
        "B_b1": _B_in["b1"],
        "B_w2": _B_in["w2"],
        "B_b2": _B_in["b2"],
    }

def reference(A_x, A_wqkv, A_wo, B_x, B_w1, B_b1, B_w2, B_b2):
    def _A_ref(x, wqkv, wo):
        B, S, D = x.shape
        H = 32; Dh = D // H
        qkv = (lambda x, *d: x.transpose(*d))((x @ wqkv).reshape(B, S, 3, H, Dh), 2, 0, 3, 1, 4)
        q, k, v = qkv[0], qkv[1], qkv[2]
        phi = lambda t: jnp.where(t > 0, t + 1, jnp.exp(t)) + 1e-6
        pq, pk = phi(q), phi(k)
        kv = jnp.einsum("bhsd,bhse->bhde", pk, v)
        z = jnp.einsum("bhsd->bhd", pk)
        num = jnp.einsum("bhqd,bhde->bhqe", pq, kv)
        den = jnp.einsum("bhqd,bhd->bhq", pq, z)[..., None] + 1e-6
        o = num / den
        return (lambda x, *d: x.transpose(*d))(o, 0, 2, 1, 3).reshape(B, S, D) @ wo

    def _B_ref(x, w1, b1, w2, b2):
        h = jnp.einsum("bsd,df->bsf", x, w1) + b1
        zero = jnp.zeros_like(h)
        r = jnp.where(h > zero, h, zero)
        h = r * r
        out = jnp.einsum("bsf,fd->bsd", h, w2) + b2
        return out

    x = A_x
    h = x + _A_ref(_layernorm(x, axis=-1), A_wqkv, A_wo)
    h2 = h + _B_ref(_layernorm(h, axis=-1), B_w1, B_b1, B_w2, B_b2)
    return h2
```

```python
import functools
import numpy as np
import jax
import jax.numpy as jnp
from jax import lax
from jax.experimental import pallas as pl
from jax.experimental.pallas import tpu as pltpu

S, D, F, H, DH = 2048, 576, 4608, 32, 18
BF, F32 = jnp.bfloat16, jnp.float32
WIN = (0, 112, 224, 336, 448)
HLO = (0, 7, 13, 19, 25)
HHI = (7, 13, 19, 25, 32)
NT = (((1,), (1,)), ((), ()))

def _ln_t(x):
    m = jnp.sum(x, axis=0, keepdims=True) * (1.0 / D)
    xc = x - m
    v = jnp.sum(xc * xc, axis=0, keepdims=True) * (1.0 / D)
    return xc * lax.rsqrt(v + 1e-5)

def _phi(t):
    return jnp.where(t > 0, t + 1.0, jnp.exp(t)) + 1e-6

def build(TS=256, NC=4, scopes=False, split_a=1, split_b=3):
    NB = S // TS
    CH = F // NC
    import contextlib
    def scope(n):
        return jax.named_scope(n) if scopes else contextlib.nullcontext()

    def kernel(x_h, wqkv_h, wo_h, w1_h, b1_h, w2t_h, b2_h, o_h,
               xs, wq_raw, wqT, wo_raw, woT, w1, w2t, b1v, b2v, ln1s, kvacc, mT, zexp, b2c, b1r,
               ln2b, hb, obuf, sems, xsems, osems):
        def xcopy(i):
            if isinstance(i, int):
                return pltpu.make_async_copy(x_h.at[:, pl.ds(i * TS, TS)], xs.at[i], xsems.at[i])
            return pltpu.make_async_copy(x_h.at[:, pl.ds(pl.multiple_of(i * TS, TS), TS)], xs.at[i], xsems.at[i])
        ckv = pltpu.make_async_copy(wqkv_h.at[:, pl.ds(512, 1216)], wq_raw.at[:, pl.ds(512, 1216)], sems.at[0])
        cq = pltpu.make_async_copy(wqkv_h.at[:, pl.ds(0, 512)], wq_raw.at[:, pl.ds(0, 512)], sems.at[1])
        co = pltpu.make_async_copy(wo_h, wo_raw, sems.at[2])
        c1 = pltpu.make_async_copy(w1_h, w1, sems.at[3])
        c2 = pltpu.make_async_copy(w2t_h, w2t, sems.at[4])
        cb1 = pltpu.make_async_copy(b1_h, b1v, sems.at[5])
        cb2 = pltpu.make_async_copy(b2_h, b2v, sems.at[6])
        with scope("start"):
            xcopy(0).start(); ckv.start(); xcopy(1).start()
            xcopy(0).wait()
            ln1s[0] = _ln_t(xs[0].astype(F32)).astype(BF)
            kvacc[...] = jnp.zeros(kvacc.shape, F32)
            ckv.wait()
            for i in range(2, NB):
                xcopy(i).start()
            cq.start(); co.start(); cb1.start(); cb2.start()
            wqT[512:, :] = wq_raw[:, 512:].T
        ones = jnp.ones((16, TS), BF)

        def p1(i, carry):
            @pl.when(i + 1 < NB)
            def _():
                xcopy(i + 1).wait()
            @pl.when(i == 1)
            def _():
                c1.start(); c2.start()
            ln = ln1s[i]
            kv = jnp.dot(wqT[D:3 * D, :], ln, preferred_element_type=F32)
            nx = jnp.minimum(i + 1, NB - 1)
            ln1s[i + 1] = _ln_t(xs[nx].astype(F32)).astype(BF)
            pk = _phi(kv[:D]).astype(BF)
            v = kv[D:].astype(BF)
            for j, a in enumerate(WIN):
                lhs = jnp.concatenate([v[a:a + 128], ones], axis=0)
                kvacc[j] += lax.dot_general(lhs, pk[a:a + 128], NT, preferred_element_type=F32)
            return carry
        with scope("p1"):
            lax.fori_loop(0, NB, p1, 0)

        with scope("mid"):
            cq.wait()
            wqT[0:512, :] = wq_raw[:, 0:512].T
            co.wait()
            for j, a in enumerate(WIN):
                woT[j] = wo_raw[a:a + 128, :].T
            cb1.wait(); cb2.wait()
            b2c[...] = jnp.broadcast_to(b2v[...].astype(F32).reshape(1, D), (128, D)).T
            b1r[...] = jnp.broadcast_to(b1v[...].astype(F32).reshape(1, F), (8, F))
            for j, a in enumerate(WIN):
                r = lax.broadcasted_iota(jnp.int32, (128, 128), 0) + a
                c = lax.broadcasted_iota(jnp.int32, (128, 128), 1) + a
                hr = (r * 3641) >> 16
                hc = (c * 3641) >> 16
                msk = (hr == hc) & (hr >= HLO[j]) & (hr < HHI[j])
                kvm = jnp.where(msk, kvacc[j, 0:128, :], 0.0).astype(BF)
                mT[j] = jnp.dot(woT[j], kvm, preferred_element_type=F32).astype(BF)
                z = kvacc[j, 128:129, :]
                zexp[j] = jnp.where(msk, jnp.broadcast_to(z, (128, 128)), 0.0).astype(BF)

        def att_q(i):
            return jnp.dot(wqT[0:D, :], ln1s[i], preferred_element_type=F32)
        def att_den(q):
            pq = _phi(q).astype(BF)
            return pq, [jnp.dot(zexp[j], pq[a:a + 128], preferred_element_type=F32) for j, a in enumerate(WIN)]
        def att_out(i, slot, pq, dens):
            att = None
            for j, a in enumerate(WIN):
                ps = (pq[a:a + 128].astype(F32) / (dens[j] + 1e-6)).astype(BF)
                t = jnp.dot(mT[j], ps, preferred_element_type=F32)
                att = t if att is None else att + t
            h = xs[i].astype(F32) + att
            ln2b[slot] = _ln_t(h).astype(BF).T
            hb[slot] = h + b2c[:, 0:1]
        def ffn1(ln2, c):
            a1 = jnp.dot(ln2, w1[:, c * CH:(c + 1) * CH], preferred_element_type=F32) + b1r[0:1, c * CH:(c + 1) * CH]
            r = jnp.maximum(a1, 0.0)
            return (r * r).astype(BF)
        def ffn2(i, slot, rs):
            r = jnp.concatenate(rs, axis=1)
            o = lax.dot_general(w2t[...], r, NT, preferred_element_type=F32)
            return (o + hb[slot]).astype(BF)
        def ocopy(i, slot):
            if isinstance(i, int):
                return pltpu.make_async_copy(obuf.at[slot], o_h.at[:, pl.ds(i * TS, TS)], osems.at[slot])
            return pltpu.make_async_copy(obuf.at[slot], o_h.at[:, pl.ds(pl.multiple_of(i * TS, TS), TS)], osems.at[slot])

        with scope("pro"):
            c1.wait(); c2.wait()
            q = att_q(0)
            pq, dens = att_den(q)
            att_out(0, 0, pq, dens)

        def p2(i, carry):
            slot = i % 2
            @pl.when(i >= 2)
            def _():
                ocopy(i - 2, slot).wait()
            ln2 = ln2b[slot]
            q = att_q(i + 1)
            rs = [ffn1(ln2, c) for c in range(split_a)]
            pq, dens = att_den(q)
            rs += [ffn1(ln2, c) for c in range(split_a, split_b)]
            att_out(i + 1, 1 - slot, pq, dens)
            rs += [ffn1(ln2, c) for c in range(split_b, NC)]
            obuf[slot] = ffn2(i, slot, rs)
            ocopy(i, slot).start()
            return carry
        with scope("p2"):
            lax.fori_loop(0, NB - 1, p2, 0)
        with scope("epi"):
            i = NB - 1
            slot = i % 2
            ocopy(i - 2, slot).wait()
            ln2 = ln2b[slot]
            rs = [ffn1(ln2, c) for c in range(NC)]
            obuf[slot] = ffn2(i, slot, rs)
            ocopy(i, slot).start()
        with scope("tail"):
            ocopy(NB - 2, (NB - 2) % 2).wait()
            ocopy(NB - 1, (NB - 1) % 2).wait()

    def fn(A_x, A_wqkv, A_wo, B_x, B_w1, B_b1, B_w2, B_b2):
        del B_x
        xt = A_x[0].T
        anyspec = pl.BlockSpec(memory_space=pl.ANY)
        ot = pl.pallas_call(
            kernel,
            out_shape=jax.ShapeDtypeStruct((D, S), BF),
            in_specs=[anyspec] * 7,
            out_specs=anyspec,
            scratch_shapes=[
                pltpu.VMEM((NB, D, TS), BF), pltpu.VMEM((D, 3 * D), BF), pltpu.VMEM((3 * D, D), BF),
                pltpu.VMEM((D, D), BF), pltpu.VMEM((5, D, 128), BF), pltpu.VMEM((D, F), BF), pltpu.VMEM((D, F), BF),
                pltpu.VMEM((F,), BF), pltpu.VMEM((D,), BF), pltpu.VMEM((NB + 1, D, TS), BF),
                pltpu.VMEM((5, 144, 128), F32), pltpu.VMEM((5, D, 128), BF), pltpu.VMEM((5, 128, 128), BF),
                pltpu.VMEM((D, 128), F32), pltpu.VMEM((8, F), F32),
                pltpu.VMEM((2, TS, D), BF), pltpu.VMEM((2, D, TS), F32), pltpu.VMEM((2, D, TS), BF),
                pltpu.SemaphoreType.DMA((7,)), pltpu.SemaphoreType.DMA((NB,)), pltpu.SemaphoreType.DMA((2,)),
            ],
            compiler_params=pltpu.CompilerParams(vmem_limit_bytes=100 * 2**20),
        )(xt, A_wqkv, A_wo, B_w1, B_b1, B_w2.T, B_b2)
        return ot.T[None]
    return fn


_FN = build()


@jax.jit
def pallas_sequential_preLN__linear_attn_block__dense_activation_squared_relu__prompt_kernel(
    A_x: jax.Array,
    A_wqkv: jax.Array,
    A_wo: jax.Array,
    B_x: jax.Array,
    B_w1: jax.Array,
    B_b1: jax.Array,
    B_w2: jax.Array,
    B_b2: jax.Array,
):
    return _FN(A_x, A_wqkv, A_wo, B_x, B_w1, B_b1, B_w2, B_b2)
```

```python
import contextlib
import numpy as np
import jax
import jax.numpy as jnp
from jax import lax
from jax.experimental import pallas as pl
from jax.experimental.pallas import tpu as pltpu

S, D, F, H, DH = 2048, 576, 4608, 32, 18
BF, F32 = jnp.bfloat16, jnp.float32
WIN = (0, 112, 224, 336, 448)
HLO = (0, 7, 13, 19, 25)
HHI = (7, 13, 19, 25, 32)
ZROW = (127, 0, 0, 0, 0)
NT = (((1,), (1,)), ((), ()))

def _phi(t):
    return jnp.where(t > 0, t + 1.0, jnp.exp(t)) + 1e-6

def _recip(d):
    r = pltpu.reciprocal(d, approx=True)
    return r * (2.0 - d * r)

def _dep_zero(a):
    b = pltpu.bitcast(a, jnp.uint32)
    return pltpu.bitcast((b >> 31) >> 1, F32)

def _finish_stats(s1, s2, c):
    s1 = jnp.sum(s1, axis=0, keepdims=True) * (1.0 / D)
    s2 = jnp.sum(s2, axis=0, keepdims=True) * (1.0 / D)
    return c + s1, lax.rsqrt(jnp.maximum(s2 - s1 * s1, 0.0) + 1e-5)

def _part_sums(d):
    R, T = d.shape
    return jnp.sum(d.reshape(R // 8, 8, T), axis=0), jnp.sum((d * d).reshape(R // 8, 8, T), axis=0)

def _expand_heads(r, T):
    rows = []
    sub = lax.broadcasted_iota(jnp.int32, (8, T), 0)
    bc = {}
    def b(h):
        if h not in bc:
            bc[h] = jnp.broadcast_to(r[h:h + 1, :], (8, T))
        return bc[h]
    for t in range(D // 8):
        h0, h1 = (8 * t) // DH, (8 * t + 7) // DH
        rows.append(b(h0) if h0 == h1 else jnp.where(sub < (h1 * DH - 8 * t), b(h0), b(h1)))
    return jnp.concatenate(rows, axis=0)

def _wins(a):
    return jnp.concatenate([a[w:w + 128] for w in WIN], axis=0)

def build(TS=256, G=2, NC=9, scopes=False, sa=0, sb=3, RC=144, RA=144, aA=(0, 1, 2, 3), aB=(5, 6, 7, 8), flags=None):
    NB = S // TS
    NG = NB // G
    CH = F // NC
    NR = D // RC
    def scope(n):
        return jax.named_scope(n) if scopes else contextlib.nullcontext()

    def kernel(x_h, wqkv_h, wo_h, w1_h, b1_h, w2t_h, b2_h, o_h,
               xs, wq_raw, wqT, wo_raw, woT, w1, w2t, b1v, b2v, lnb, pqs, kvacc, mT, zw, msks, zmsk, b2c, b1r,
               ln2b, hb, obuf, sems, osems):
        def dyn(i, n):
            return i * n if isinstance(i, int) else pl.multiple_of(i * n, n)
        def xcopy(i):
            return pltpu.make_async_copy(x_h.at[:, pl.ds(dyn(i, TS), TS)], xs.at[i], sems.at[8 + i])
        def ocopy(i):
            return pltpu.make_async_copy(obuf.at[i], o_h.at[:, pl.ds(dyn(i, TS), TS)], osems.at[i])
        def wcopy(k, lo, n):
            return pltpu.make_async_copy(wqkv_h.at[:, pl.ds(lo, n)], wq_raw.at[:, pl.ds(lo, n)], sems.at[k])
        cwa, cwb, cwc = wcopy(0, 512, 640), wcopy(1, 1152, 576), wcopy(7, 0, 512)
        co = pltpu.make_async_copy(wo_h, wo_raw, sems.at[2])
        c1 = pltpu.make_async_copy(w1_h, w1, sems.at[3])
        c2 = pltpu.make_async_copy(w2t_h, w2t, sems.at[4])
        cb1 = pltpu.make_async_copy(b1_h, b1v, sems.at[5])
        cb2 = pltpu.make_async_copy(b2_h, b2v, sems.at[6])

        def with_ones(v, j):
            w, u = WIN[j], ZROW[j]
            g = (u // 16) * 16
            sel = lax.broadcasted_iota(jnp.int32, (16, TS), 0) == (u - g)
            mid = jnp.where(sel, jnp.ones((16, TS), BF), v[w + g:w + g + 16])
            parts = ([v[w:w + g]] if g > 0 else []) + [mid] + ([v[w + g + 16:w + 128]] if g + 16 < 128 else [])
            return jnp.concatenate(parts, axis=0)

        def ln_plain(b):
            xf = xs[b].astype(F32)
            c = xf[0:1, :]
            m, rstd = _finish_stats(*_part_sums(xf - c), c)
            return ((xf - m) * rstd).astype(BF)

        def ln_stats(b, anch):
            R = D // len(anch)
            c = xs[b, 0:16, :].astype(F32)[0:1]
            s1 = s2 = None
            for g, a in enumerate(anch):
                t1, t2 = _part_sums(xs[b, g * R:(g + 1) * R, :].astype(F32) - (c + _dep_zero(a)[0:1]))
                s1, s2 = (t1, t2) if s1 is None else (s1 + t1, s2 + t2)
            return _finish_stats(s1, s2, c)

        def ln_store(b, slot, m, rstd, anch):
            R = D // len(anch)
            for g, a in enumerate(anch):
                lnb[slot, g * R:(g + 1) * R, :] = (
                    (xs[b, g * R:(g + 1) * R, :].astype(F32) - (m + _dep_zero(a)[0:1])) * rstd).astype(BF)

        def kv_dots(pk, v, first):
            for j, w in enumerate(WIN):
                t = lax.dot_general(with_ones(v, j), pk[w:w + 128], NT, preferred_element_type=F32)
                kvacc[j] = t if first else kvacc[j] + t

        def proj(lo, c, ln):
            return jnp.dot(wqT[lo + c * RC:lo + (c + 1) * RC, :], ln, preferred_element_type=F32)

        def p1_block(i, slot, ln, nxt, nslot):
            res = [proj(D, c, ln) for c in range(NR)]
            pk = _phi(jnp.concatenate(res, axis=0)).astype(BF)
            res += [proj(2 * D, c, ln) for c in range(NR)]
            v = jnp.concatenate(res[NR:], axis=0).astype(BF)
            m, rstd = ln_stats(nxt, [res[a][0:8] for a in aA])
            res += [proj(0, c, ln) for c in range(NR)]
            kv_dots(pk, v, False)
            ln_store(nxt, nslot, m, rstd, [res[a][0:8] for a in aB])
            pqs[i] = _phi(jnp.concatenate(res[2 * NR:], axis=0)).astype(BF)

        def build_att_consts():
            for j, w in enumerate(WIN):
                z = kvacc[j, ZROW[j]:ZROW[j] + 1, :]
                zw[:, 128 * j:128 * j + 128] = (zmsk[:, 128 * j:128 * j + 128] * jnp.broadcast_to(z, (32, 128))).astype(BF)
        def build_mT():
            for j, w in enumerate(WIN):
                kvm = jnp.where(msks[j] > 0.5, kvacc[j], 0.0).astype(BF)
                for c in range(D // RA):
                    mT[c * RA:(c + 1) * RA, 128 * j:128 * j + 128] = jnp.dot(
                        woT[j, c * RA:(c + 1) * RA, :], kvm, preferred_element_type=F32).astype(BF)
        def att_den(i):
            pq = pqs[i]
            return pq, jnp.dot(zw[...], _wins(pq), preferred_element_type=F32)
        def att_ps(pq, den):
            return (pq.astype(F32) * _expand_heads(_recip(den + 1e-6), TS)).astype(BF)
        def att_dot(ps):
            psw = _wins(ps)
            return jnp.concatenate([jnp.dot(mT[c * RA:(c + 1) * RA, :], psw, preferred_element_type=F32)
                                    for c in range(D // RA)], axis=0)
        def att_fin(i, slot, att):
            h = xs[i].astype(F32) + att
            hb[slot] = h
            c = h[0:1, :]
            m, rstd = _finish_stats(*_part_sums(h - c), c)
            ln2b[slot] = ((hb[slot] - m) * rstd).astype(BF).T
        def ffn1(ln2, c):
            a1 = jnp.dot(ln2, w1[:, c * CH:(c + 1) * CH], preferred_element_type=F32) + b1r[0:1, c * CH:(c + 1) * CH]
            r = jnp.maximum(a1, 0.0)
            return (r * r).astype(BF)
        def ffn2(i, slot, rs):
            r = jnp.concatenate(rs, axis=1)
            o = lax.dot_general(w2t[...], r, NT, preferred_element_type=F32)
            obuf[i] = (o + (hb[slot] + b2c[:, 0:1])).astype(BF)
            ocopy(i).start()
        def p2_block(i, slot, with_att=True):
            ln2 = ln2b[slot]
            if not with_att:
                ffn2(i, slot, [ffn1(ln2, c) for c in range(NC)])
                return
            rs = [ffn1(ln2, c) for c in range(sa)]
            ps = att_ps(*att_den(i + 1))
            rs += [ffn1(ln2, c) for c in range(sa, sb)]
            att_fin(i + 1, 1 - slot, att_dot(ps))
            rs += [ffn1(ln2, c) for c in range(sb, NC)]
            ffn2(i, slot, rs)

        with scope("start"):
            first = [xcopy(0), cb1, cb2, cwa] + [xcopy(b) for b in range(1, G)] + [cwb, cwc, xcopy(G), co]
            for c in first:
                c.start()
            for b in range(G + 1, NB):
                xcopy(b).start()
            c1.start(); c2.start()
            for j, w in enumerate(WIN):
                r = lax.broadcasted_iota(jnp.int32, (128, 128), 0) + w
                c = lax.broadcasted_iota(jnp.int32, (128, 128), 1) + w
                hr, hc = (r * 3641) >> 16, (c * 3641) >> 16
                msks[j] = jnp.where((hr == hc) & (hr >= HLO[j]) & (hr < HHI[j]), 1.0, 0.0)
                hsel = lax.broadcasted_iota(jnp.int32, (32, 128), 0)
                hd = ((lax.broadcasted_iota(jnp.int32, (32, 128), 1) + w) * 3641) >> 16
                zmsk[:, 128 * j:128 * j + 128] = jnp.where((hd == hsel) & (hd >= HLO[j]) & (hd < HHI[j]), 1.0, 0.0)
            with scope("w_x0"):
                xcopy(0).wait(); cb1.wait(); cb2.wait()
            lnb[0] = ln_plain(0)
            b2c[...] = jnp.broadcast_to(b2v[...].astype(F32).reshape(1, D), (128, D)).T
            b1r[...] = jnp.broadcast_to(b1v[...].astype(F32).reshape(1, F), (8, F))
            with scope("w_a"):
                cwa.wait()
            wqT[512:1152, :] = wq_raw[:, 512:1152].T
            with scope("w_x1"):
                for b in range(1, G):
                    xcopy(b).wait()
            pks = []
            lns = [lnb[0]]
            for b in range(G):
                if b == G - 1:
                    with scope("w_b"):
                        cwb.wait()
                    lns = [lnb[u] for u in range(G)]
                kk = [proj(D, c, lns[b]) for c in range(NR)]
                if b + 1 < G:
                    m, rstd = ln_stats(b + 1, [kk[0][0:8], kk[0][0:8], kk[1][0:8], kk[1][0:8]])
                    kvacc[0, 0:8, :] = jnp.zeros((8, 128), F32)
                    ln_store(b + 1, b + 1, m, rstd, [kk[2][0:8], kk[2][0:8], kk[3][0:8], kk[3][0:8]])
                pks.append(_phi(jnp.concatenate(kk, axis=0)).astype(BF))
            wqT[1152:1728, :] = wq_raw[:, 1152:1728].T
            with scope("w_c"):
                cwc.wait(); xcopy(G).wait()
            lns = [lnb[u] for u in range(G)]
            vs = [jnp.concatenate([proj(2 * D, c, lns[b]) for c in range(NR)], axis=0) for b in range(G)]
            wt = wq_raw[:, 0:512].T
            wqT[0:512, :] = wt
            wq = jnp.concatenate([wt, wqT[512:576, :]], axis=0)
            m, rstd = ln_stats(G, [vs[0][a * RC:a * RC + 8] for a in range(4)])
            qs = []
            for b in range(G):
                qs.append(jnp.concatenate([jnp.dot(wq[c * RC:(c + 1) * RC], lns[b], preferred_element_type=F32)
                                           for c in range(NR)], axis=0))
                kv_dots(pks[b], vs[b].astype(BF), b == 0)
                pqs[b] = _phi(qs[b]).astype(BF)
            ln_store(G, G, m, rstd, [qs[0][a * RC:a * RC + 8] for a in range(4)])

        co.wait()
        def p1(g, carry):
            @pl.when(g + 1 < NG)
            def _():
                for u in range(1, G + 1):
                    xcopy(g * G + u).wait()
            @pl.when(g + 1 == NG)
            def _():
                for u in range(1, G):
                    xcopy(g * G + u).wait()
            par = g % 2
            jw0 = (g - 1) * WPI
            for u in range(WPI):
                jw = jnp.minimum(jw0 + u, 4)
                woT[jw] = wo_raw[pl.ds(pl.multiple_of(jw * 112, 16), 128), :].T
            for u in range(G):
                b = g * G + u
                nslot = par * G + u + 1 if u + 1 < G else (1 - par) * G
                p1_block(b, None, lnb[par * G + u], jnp.minimum(b + 1, NB - 1), nslot)
            return carry
        WPI = -(-5 // (NG - 1))
        with scope("p1"):
            lax.fori_loop(1, NG, p1, 0)

        with scope("mid"):
            c1.wait(); c2.wait()
            build_att_consts()
            d0 = att_den(0)
            build_mT()
            att_fin(0, 0, att_dot(att_ps(*d0)))

        with scope("p2"):
            lax.fori_loop(0, NB - 1, lambda i, c: (p2_block(i, i % 2), c)[1], 0)
        with scope("epi"):
            p2_block(NB - 1, (NB - 1) % 2, with_att=False)
        with scope("tail"):
            for b in range(NB):
                ocopy(b).wait()

    def fn(A_x, A_wqkv, A_wo, B_x, B_w1, B_b1, B_w2, B_b2):
        del B_x
        xt = A_x[0].T
        anyspec = pl.BlockSpec(memory_space=pl.ANY)
        ot = pl.pallas_call(
            kernel,
            out_shape=jax.ShapeDtypeStruct((D, S), BF),
            in_specs=[anyspec] * 7,
            out_specs=anyspec,
            scratch_shapes=[
                pltpu.VMEM((NB, D, TS), BF), pltpu.VMEM((D, 3 * D), BF), pltpu.VMEM((3 * D, D), BF),
                pltpu.VMEM((D, D), BF), pltpu.VMEM((5, D, 128), BF), pltpu.VMEM((D, F), BF), pltpu.VMEM((D, F), BF),
                pltpu.VMEM((F,), BF), pltpu.VMEM((D,), BF), pltpu.VMEM((2 * G, D, TS), BF), pltpu.VMEM((NB, D, TS), BF),
                pltpu.VMEM((5, 128, 128), F32), pltpu.VMEM((D, 640), BF), pltpu.VMEM((32, 640), BF),
                pltpu.VMEM((5, 128, 128), F32), pltpu.VMEM((32, 640), F32),
                pltpu.VMEM((D, 128), F32), pltpu.VMEM((8, F), F32),
                pltpu.VMEM((2, TS, D), BF), pltpu.VMEM((2, D, TS), F32), pltpu.VMEM((NB, D, TS), BF),
                pltpu.SemaphoreType.DMA((8 + NB,)), pltpu.SemaphoreType.DMA((NB,)),
            ],
            compiler_params=pltpu.CompilerParams(vmem_limit_bytes=110 * 2**20, flags=flags),
        )(xt, A_wqkv, A_wo, B_w1, B_b1, B_w2.T, B_b2)
        return ot.T[None]
    return fn


_FN = build()


@jax.jit
def pallas_sequential_preLN__linear_attn_block__dense_activation_squared_relu__prompt_kernel(
    A_x: jax.Array,
    A_wqkv: jax.Array,
    A_wo: jax.Array,
    B_x: jax.Array,
    B_w1: jax.Array,
    B_b1: jax.Array,
    B_w2: jax.Array,
    B_b2: jax.Array,
):
    return _FN(A_x, A_wqkv, A_wo, B_x, B_w1, B_b1, B_w2, B_b2)
```

```python
import contextlib
import numpy as np
import jax
import jax.numpy as jnp
from jax import lax
from jax.experimental import pallas as pl
from jax.experimental.pallas import tpu as pltpu

S, D, F, H, DH = 2048, 576, 4608, 32, 18
BF, F32 = jnp.bfloat16, jnp.float32
WIN = (0, 112, 224, 336, 448)
HLO = (0, 7, 13, 19, 25)
HHI = (7, 13, 19, 25, 32)
ZROW = (127, 0, 0, 0, 0)
NT = (((1,), (1,)), ((), ()))

def _phi(t):
    return jnp.where(t > 0, t + 1.0, jnp.exp(t)) + 1e-6

def _recip(d):
    r = pltpu.reciprocal(d, approx=True)
    return r * (2.0 - d * r)

def _dep_zero(a):
    b = pltpu.bitcast(a, jnp.uint32)
    return pltpu.bitcast((b >> 31) >> 1, F32)

def _finish_stats(s1, s2, c):
    s1 = jnp.sum(s1, axis=0, keepdims=True) * (1.0 / D)
    s2 = jnp.sum(s2, axis=0, keepdims=True) * (1.0 / D)
    return c + s1, lax.rsqrt(jnp.maximum(s2 - s1 * s1, 0.0) + 1e-5)

def _part_sums(d):
    R, T = d.shape
    return jnp.sum(d.reshape(R // 8, 8, T), axis=0), jnp.sum((d * d).reshape(R // 8, 8, T), axis=0)

def _expand_heads(r, T):
    rows = []
    sub = lax.broadcasted_iota(jnp.int32, (8, T), 0)
    bc = {}
    def b(h):
        if h not in bc:
            bc[h] = jnp.broadcast_to(r[h:h + 1, :], (8, T))
        return bc[h]
    for t in range(D // 8):
        h0, h1 = (8 * t) // DH, (8 * t + 7) // DH
        rows.append(b(h0) if h0 == h1 else jnp.where(sub < (h1 * DH - 8 * t), b(h0), b(h1)))
    return jnp.concatenate(rows, axis=0)

def _wins(a):
    return jnp.concatenate([a[w:w + 128] for w in WIN], axis=0)

def build(TS=256, G=2, NC=9, scopes=False, sa=0, sb=3, RC=144, RA=144, aA=(0, 1, 2, 3), aB=(5, 6, 7, 8), peel_last=False, manch=(-1,-1,0,280,568), halves=False, morder='qzdqmqaqqqqqf', esplit=4, G1=2, mxt=0, SA=0, flags=None):
    NB = S // TS
    NG = NB // G
    CH = F // NC
    NR = D // RC
    def scope(n):
        return jax.named_scope(n) if scopes else contextlib.nullcontext()

    def kernel(x_h, wqkv_h, wo_h, w1_h, b1_h, w2t_h, b2_h, o_h,
               xs, wq_raw, wqT, wo_raw, woT, w1, w2t, b1v, b2v, lnb, pqs, kvacc, mT, zw, msks, zmsk, b2c, b1r,
               ln2b, hb, obuf, sems, osems, esems):
        def dyn(i, n):
            return i * n if isinstance(i, int) else pl.multiple_of(i * n, n)
        def xcopy(i):
            return pltpu.make_async_copy(x_h.at[:, pl.ds(dyn(i, TS), TS)], xs.at[i], sems.at[8 + i])
        def ocopy(i):
            return pltpu.make_async_copy(obuf.at[i], o_h.at[:, pl.ds(dyn(i, TS), TS)], osems.at[i])
        def wcopy(k, lo, n):
            return pltpu.make_async_copy(wqkv_h.at[:, pl.ds(lo, n)], wq_raw.at[:, pl.ds(lo, n)], sems.at[k])
        cwa, cwb, cwc = wcopy(0, 512, (SA or 1152) - 512), wcopy(1, 1152, 576), wcopy(7, 0, 512)
        cwa2 = pltpu.make_async_copy(wqkv_h.at[:, pl.ds(SA, 1152 - SA)], wq_raw.at[:, pl.ds(SA, 1152 - SA)], esems.at[7]) if SA else None
        co = pltpu.make_async_copy(wo_h, wo_raw, sems.at[2])
        c1 = pltpu.make_async_copy(w1_h, w1, sems.at[3])
        c2 = pltpu.make_async_copy(w2t_h, w2t, sems.at[4])
        cb1 = pltpu.make_async_copy(b1_h, b1v, sems.at[5])
        cb2 = pltpu.make_async_copy(b2_h, b2v, sems.at[6])

        def with_ones(v, j):
            w, u = WIN[j], ZROW[j]
            g = (u // 16) * 16
            sel = lax.broadcasted_iota(jnp.int32, (16, TS), 0) == (u - g)
            mid = jnp.where(sel, jnp.ones((16, TS), BF), v[w + g:w + g + 16])
            parts = ([v[w:w + g]] if g > 0 else []) + [mid] + ([v[w + g + 16:w + 128]] if g + 16 < 128 else [])
            return jnp.concatenate(parts, axis=0)

        def ln_plain(b):
            xf = xs[b].astype(F32)
            c = xf[0:1, :]
            m, rstd = _finish_stats(*_part_sums(xf - c), c)
            return ((xf - m) * rstd).astype(BF)

        def ln_stats(b, anch):
            R = D // len(anch)
            c = xs[b, 0:16, :].astype(F32)[0:1]
            s1 = s2 = None
            for g, a in enumerate(anch):
                t1, t2 = _part_sums(xs[b, g * R:(g + 1) * R, :].astype(F32) - (c + _dep_zero(a)[0:1]))
                s1, s2 = (t1, t2) if s1 is None else (s1 + t1, s2 + t2)
            return _finish_stats(s1, s2, c)

        def ln_store(b, slot, m, rstd, anch):
            R = D // len(anch)
            for g, a in enumerate(anch):
                lnb[slot, g * R:(g + 1) * R, :] = (
                    (xs[b, g * R:(g + 1) * R, :].astype(F32) - (m + _dep_zero(a)[0:1])) * rstd).astype(BF)

        def kv_dots(pk, v, first):
            for j, w in enumerate(WIN):
                t = lax.dot_general(with_ones(v, j), pk[w:w + 128], NT, preferred_element_type=F32)
                kvacc[j] = t if first else kvacc[j] + t

        def proj(lo, c, ln):
            return jnp.dot(wqT[lo + c * RC:lo + (c + 1) * RC, :], ln, preferred_element_type=F32)

        def p1_block(i, nxt, nslot):
            ln = lnb[i]
            res = [proj(D, c, ln) for c in range(NR)]
            pk = _phi(jnp.concatenate(res, axis=0)).astype(BF)
            res += [proj(2 * D, c, ln) for c in range(NR)]
            v = jnp.concatenate(res[NR:], axis=0).astype(BF)
            m, rstd = ln_stats(nxt, [res[a][0:8] for a in aA])
            lq = lnb[i - G]
            res += [proj(0, c, lq) for c in range(NR)]
            kv_dots(pk, v, False)
            ln_store(nxt, nslot, m, rstd, [res[a][0:8] for a in aB])
            pqs[i - G] = _phi(jnp.concatenate(res[2 * NR:], axis=0)).astype(BF)

        def build_att_consts():
            for j, w in enumerate(WIN):
                z = kvacc[j, ZROW[j]:ZROW[j] + 1, :]
                zw[:, 128 * j:128 * j + 128] = (zmsk[:, 128 * j:128 * j + 128] * jnp.broadcast_to(z, (32, 128))).astype(BF)
        def build_mT(anch=None):
            for j, w in enumerate(WIN):
                kvm = jnp.where(msks[j] > 0.5, kvacc[j], 0.0)
                if anch is not None and anch[j] is not None:
                    kvm = kvm + _dep_zero(anch[j])[0:1, 0:128]
                kvm = kvm.astype(BF)
                for c in range(D // RA):
                    mT[c * RA:(c + 1) * RA, 128 * j:128 * j + 128] = jnp.dot(
                        woT[j, c * RA:(c + 1) * RA, :], kvm, preferred_element_type=F32).astype(BF)
        def att_den(i):
            pq = pqs[i]
            return pq, jnp.dot(zw[...], _wins(pq), preferred_element_type=F32)
        def att_ps(pq, den):
            return (pq.astype(F32) * _expand_heads(_recip(den + 1e-6), TS)).astype(BF)
        def att_dot(ps):
            psw = _wins(ps)
            return jnp.concatenate([jnp.dot(mT[c * RA:(c + 1) * RA, :], psw, preferred_element_type=F32)
                                    for c in range(D // RA)], axis=0)
        def att_fin(i, slot, att):
            h = xs[i].astype(F32) + att
            hb[slot] = h
            c = h[0:1, :]
            m, rstd = _finish_stats(*_part_sums(h - c), c)
            ln2b[slot] = ((hb[slot] - m) * rstd).astype(BF).T
        def ffn1(ln2, c):
            a1 = jnp.dot(ln2, w1[:, c * CH:(c + 1) * CH], preferred_element_type=F32) + b1r[0:1, c * CH:(c + 1) * CH]
            r = jnp.maximum(a1, 0.0)
            return (r * r).astype(BF)
        def ffn2(i, slot, rs):
            r = jnp.concatenate(rs, axis=1)
            o = lax.dot_general(w2t[...], r, NT, preferred_element_type=F32)
            obuf[i] = (o + (hb[slot] + b2c[:, 0:1])).astype(BF)
            ocopy(i).start()
        def p2_block(i, slot, with_att=True):
            ln2 = ln2b[slot]
            if not with_att:
                ffn2(i, slot, [ffn1(ln2, c) for c in range(NC)])
                return
            rs = [ffn1(ln2, c) for c in range(sa)]
            ps = att_ps(*att_den(i + 1))
            rs += [ffn1(ln2, c) for c in range(sa, sb)]
            att_fin(i + 1, 1 - slot, att_dot(ps))
            rs += [ffn1(ln2, c) for c in range(sb, NC)]
            ffn2(i, slot, rs)

        with scope("start"):
            first = [xcopy(0), cb1, cb2, cwa] + [xcopy(b) for b in range(1, G)] + ([cwa2] if SA else []) + [cwb, cwc, xcopy(G), co]
            for c in first:
                c.start()
            for b in range(G + 1, NB):
                xcopy(b).start()
            c1.start(); c2.start()
            for j, w in enumerate(WIN):
                r = lax.broadcasted_iota(jnp.int32, (128, 128), 0) + w
                c = lax.broadcasted_iota(jnp.int32, (128, 128), 1) + w
                hr, hc = (r * 3641) >> 16, (c * 3641) >> 16
                msks[j] = jnp.where((hr == hc) & (hr >= HLO[j]) & (hr < HHI[j]), 1.0, 0.0)
                hsel = lax.broadcasted_iota(jnp.int32, (32, 128), 0)
                hd = ((lax.broadcasted_iota(jnp.int32, (32, 128), 1) + w) * 3641) >> 16
                zmsk[:, 128 * j:128 * j + 128] = jnp.where((hd == hsel) & (hd >= HLO[j]) & (hd < HHI[j]), 1.0, 0.0)
            with scope("w_x0"):
                xcopy(0).wait(); cb1.wait(); cb2.wait()
            lnb[0] = ln_plain(0)
            b2c[...] = jnp.broadcast_to(b2v[...].astype(F32).reshape(1, D), (128, D)).T
            b1r[...] = jnp.broadcast_to(b1v[...].astype(F32).reshape(1, F), (8, F))
            if SA == 0:
                with scope("w_a"):
                    cwa.wait()
                if mxt:
                    eye = (lax.broadcasted_iota(jnp.int32, (128, 128), 0) == lax.broadcasted_iota(jnp.int32, (128, 128), 1)).astype(BF)
                    for t in range(5 - mxt, 5):
                        lo = 512 + 128 * t
                        wqT[lo:lo + 128, :] = lax.dot_general(eye, wq_raw[:, lo:lo + 128], NT, preferred_element_type=F32).astype(BF)
                hi = 1152 - 128 * mxt
                wqT[512:hi, :] = wq_raw[:, 512:hi].T
                with scope("w_x1"):
                    for b in range(1, G):
                        xcopy(b).wait()
                pks = []
                lns = [lnb[0]]
                for b in range(G):
                    if b == G - 1:
                        with scope("w_b"):
                            cwb.wait()
                        lns = [lnb[u] for u in range(G)]
                    kk = [proj(D, c, lns[b]) for c in range(NR)]
                    if b + 1 < G:
                        m, rstd = ln_stats(b + 1, [kk[0][0:8], kk[0][0:8], kk[1][0:8], kk[1][0:8]])
                        kvacc[0, 0:8, :] = jnp.zeros((8, 128), F32)
                        ln_store(b + 1, b + 1, m, rstd, [kk[2][0:8], kk[2][0:8], kk[3][0:8], kk[3][0:8]])
                    pks.append(_phi(jnp.concatenate(kk, axis=0)).astype(BF))
                wqT[1152:1728, :] = wq_raw[:, 1152:1728].T
            else:
                def kd(lo, hi, ln):
                    return jnp.dot(wqT[lo:hi, :], ln, preferred_element_type=F32)
                with scope("w_a"):
                    cwa.wait()
                wqT[512:SA, :] = wq_raw[:, 512:SA].T
                with scope("w_x1"):
                    xcopy(1).wait()
                h1 = (576 + SA) // 2 // 16 * 16
                ka0 = [kd(576, h1, lnb[0]), kd(h1, SA, lnb[0])]
                m, rstd = ln_stats(1, [ka0[0][0:8]] * 4)
                kvacc[0, 0:8, :] = jnp.zeros((8, 128), F32)
                ln_store(1, 1, m, rstd, [ka0[0][0:8]] * 4)
                ln1 = lnb[1]
                ka1 = [kd(576, h1, ln1), kd(h1, SA, ln1)]
                pa = [_phi(jnp.concatenate(ka0, axis=0)).astype(BF), _phi(jnp.concatenate(ka1, axis=0)).astype(BF)]
                with scope("w_a2"):
                    cwa2.wait()
                wqT[SA:1152, :] = wq_raw[:, SA:1152].T
                with scope("w_b"):
                    cwb.wait()
                h2 = (SA + 1152) // 2 // 16 * 16
                pks = []
                for b in range(2):
                    ln = lnb[b]
                    kb = [kd(SA, h2, ln), kd(h2, 1152, ln)]
                    pks.append(jnp.concatenate([pa[b], _phi(jnp.concatenate(kb, axis=0)).astype(BF)], axis=0))
                wqT[1152:1728, :] = wq_raw[:, 1152:1728].T
            with scope("w_c"):
                cwc.wait(); xcopy(G).wait()
            lns = [lnb[u] for u in range(G)]
            vs = [jnp.concatenate([proj(2 * D, c, lns[b]) for c in range(NR)], axis=0) for b in range(G)]
            wqT[0:512, :] = wq_raw[:, 0:512].T
            m, rstd = ln_stats(G, [vs[0][a * RC:a * RC + 8] for a in range(4)])
            for b in range(G):
                kv_dots(pks[b], vs[b].astype(BF), b == 0)
            ln_store(G, G, m, rstd, [vs[G - 1][a * RC:a * RC + 8] for a in range(4)])

        co.wait()
        def p1(g, carry):
            b0 = G + g * G1
            @pl.when(g + 1 < NG1)
            def _():
                for u in range(1, G1 + 1):
                    xcopy(b0 + u).wait()
            @pl.when(g + 1 == NG1)
            def _():
                for u in range(1, G1):
                    xcopy(b0 + u).wait()
            jw0 = g * WPI
            for u in range(WPI):
                jw = jnp.minimum(jw0 + u, 4)
                woT[jw] = wo_raw[pl.ds(pl.multiple_of(jw * 112, 16), 128), :].T
            for u in range(G1):
                b = b0 + u
                p1_block(b, jnp.minimum(b + 1, NB - 1), b + 1)
            return carry
        NG1 = (NB - G) // G1
        WPI = -(-5 // NG1)
        with scope("p1"):
            lax.fori_loop(0, NG1, p1, 0)

        with scope("mid"):
            c1.wait(); c2.wait()
            qs = [[] for _ in range(G)]
            lq = [lnb[NB - G + u] for u in range(G)]
            st = {}
            def qn():
                for u in range(G):
                    if len(qs[u]) < NR:
                        qs[u].append(proj(0, len(qs[u]), lq[u]))
                        if len(qs[u]) == NR:
                            pqs[NB - G + u] = _phi(jnp.concatenate(qs[u], axis=0)).astype(BF)
                        return
            for ch in morder:
                if ch == 'q': qn()
                elif ch == 'z': build_att_consts()
                elif ch == 'M': build_mT()
                elif ch == 'd': st['d'] = att_den(0)
                elif ch == 'm':
                    pq, den = st['d']
                    st['ps'] = pq.astype(F32) * _expand_heads(_recip(den + 1e-6), TS)
                    build_mT([None if a < 0 else st['ps'][a:a + 8] for a in manch])
                elif ch == 'a': st['a'] = att_dot(st['ps'].astype(BF) if 'ps' in st else att_ps(*st['d']))
                elif ch == 'f': att_fin(0, 0, st['a'])
            assert all(len(q) == NR for q in qs)

        with scope("p2"):
            lax.fori_loop(0, NB - 1, lambda i, c: (p2_block(i, i % 2), c)[1], 0)
        with scope("epi"):
            last = []
            if esplit == 0:
                p2_block(NB - 1, (NB - 1) % 2, with_att=False)
                last.append(ocopy(NB - 1))
            else:
                i, slot = NB - 1, (NB - 1) % 2
                ln2 = ln2b[slot]
                r = jnp.concatenate([ffn1(ln2, c) for c in range(NC)], axis=1)
                k = 0
                for u in range(TS // 128):
                    nr = 1 if (u + 1 < TS // 128) else esplit
                    R = D // nr
                    for c in range(nr):
                        o = lax.dot_general(w2t[c * R:(c + 1) * R, :], r[128 * u:128 * u + 128], NT, preferred_element_type=F32)
                        obuf[i, c * R:(c + 1) * R, 128 * u:128 * u + 128] = (
                            o + (hb[slot, c * R:(c + 1) * R, 128 * u:128 * u + 128] + b2c[c * R:(c + 1) * R, 0:1])).astype(BF)
                        cp = pltpu.make_async_copy(obuf.at[i, pl.ds(c * R, R), pl.ds(128 * u, 128)],
                                                   o_h.at[pl.ds(c * R, R), pl.ds(i * TS + 128 * u, 128)], esems.at[k])
                        cp.start()
                        last.append(cp)
                        k += 1
        with scope("tail"):
            for b in range(NB - 1):
                ocopy(b).wait()
            for cp in last:
                cp.wait()

    def fn(A_x, A_wqkv, A_wo, B_x, B_w1, B_b1, B_w2, B_b2):
        del B_x
        xt = A_x[0].T
        anyspec = pl.BlockSpec(memory_space=pl.ANY)
        ot = pl.pallas_call(
            kernel,
            out_shape=jax.ShapeDtypeStruct((D, S), BF),
            in_specs=[anyspec] * 7,
            out_specs=anyspec,
            scratch_shapes=[
                pltpu.VMEM((NB, D, TS), BF), pltpu.VMEM((D, 3 * D), BF), pltpu.VMEM((3 * D, D), BF),
                pltpu.VMEM((D, D), BF), pltpu.VMEM((5, D, 128), BF), pltpu.VMEM((D, F), BF), pltpu.VMEM((D, F), BF),
                pltpu.VMEM((F,), BF), pltpu.VMEM((D,), BF), pltpu.VMEM((NB + 1, D, TS), BF), pltpu.VMEM((NB, D, TS), BF),
                pltpu.VMEM((5, 128, 128), F32), pltpu.VMEM((D, 640), BF), pltpu.VMEM((32, 640), BF),
                pltpu.VMEM((5, 128, 128), F32), pltpu.VMEM((32, 640), F32),
                pltpu.VMEM((D, 128), F32), pltpu.VMEM((8, F), F32),
                pltpu.VMEM((2, TS, D), BF), pltpu.VMEM((2, D, TS), F32), pltpu.VMEM((NB, D, TS), BF),
                pltpu.SemaphoreType.DMA((8 + NB,)), pltpu.SemaphoreType.DMA((NB,)),
                pltpu.SemaphoreType.DMA((8,)),
            ],
            compiler_params=pltpu.CompilerParams(vmem_limit_bytes=110 * 2**20, flags=flags),
        )(xt, A_wqkv, A_wo, B_w1, B_b1, B_w2.T, B_b2)
        return ot.T[None]
    return fn


_FN = build()


@jax.jit
def pallas_sequential_preLN__linear_attn_block__dense_activation_squared_relu__prompt_kernel(
    A_x: jax.Array,
    A_wqkv: jax.Array,
    A_wo: jax.Array,
    B_x: jax.Array,
    B_w1: jax.Array,
    B_b1: jax.Array,
    B_w2: jax.Array,
    B_b2: jax.Array,
):
    return _FN(A_x, A_wqkv, A_wo, B_x, B_w1, B_b1, B_w2, B_b2)
```

```python
import jax
import jax.numpy as jnp
from jax import lax
from jax.experimental import pallas as pl
from jax.experimental.pallas import tpu as pltpu

S, D, F, DH = 2048, 576, 4608, 18
BF, F32 = jnp.bfloat16, jnp.float32
TS = 256
NB = S // TS
G = 2
RC = 144
NR = D // RC
NC = 9
CH = F // NC
WIN = (0, 112, 224, 336, 448)
HLO = (0, 7, 13, 19, 25)
HHI = (7, 13, 19, 25, 32)
ZROW = (127, 0, 0, 0, 0)
NT = (((1,), (1,)), ((), ()))


def _phi(t):
    return jnp.where(t > 0, t + 1.0, jnp.exp(t)) + 1e-6


def _recip(d):
    r = pltpu.reciprocal(d, approx=True)
    return r * (2.0 - d * r)


def _dep_zero(a):
    b = pltpu.bitcast(a, jnp.uint32)
    return pltpu.bitcast((b >> 31) >> 1, F32)


def _part_sums(d):
    r, t = d.shape
    return (jnp.sum(d.reshape(r // 8, 8, t), axis=0),
            jnp.sum((d * d).reshape(r // 8, 8, t), axis=0))


def _ln_stats(s1, s2, c):
    s1 = jnp.sum(s1, axis=0, keepdims=True) * (1.0 / D)
    s2 = jnp.sum(s2, axis=0, keepdims=True) * (1.0 / D)
    return c + s1, lax.rsqrt(jnp.maximum(s2 - s1 * s1, 0.0) + 1e-5)


def _expand_heads(r):
    t = r.shape[1]
    sub = lax.broadcasted_iota(jnp.int32, (8, t), 0)
    bc = {}

    def b(h):
        if h not in bc:
            bc[h] = jnp.broadcast_to(r[h:h + 1, :], (8, t))
        return bc[h]

    rows = []
    for g in range(D // 8):
        h0, h1 = (8 * g) // DH, (8 * g + 7) // DH
        rows.append(b(h0) if h0 == h1 else jnp.where(sub < (h1 * DH - 8 * g), b(h0), b(h1)))
    return jnp.concatenate(rows, axis=0)


def _wins(a):
    return jnp.concatenate([a[w:w + 128] for w in WIN], axis=0)


def _head_of(i):
    return (i * 3641) >> 16


def _dyn(i, n):
    return i * n if isinstance(i, int) else pl.multiple_of(i * n, n)


def _kernel(x_h, wqkv_h, wo_h, w1_h, b1_h, w2t_h, b2_h, o_h,
            xs, wq_raw, wqT, wo_raw, woT, w1, w2t, b1v, b2v, lnb, pqs, kvacc, mT, zw, msks, zmsk,
            b2c, b1r, ln2b, hb, obuf, sems, osems, esems):
    def xcopy(i):
        return pltpu.make_async_copy(x_h.at[:, pl.ds(_dyn(i, TS), TS)], xs.at[i], sems.at[8 + i])

    def ocopy(i):
        return pltpu.make_async_copy(obuf.at[i], o_h.at[:, pl.ds(_dyn(i, TS), TS)], osems.at[i])

    def wcopy(k, lo, n):
        return pltpu.make_async_copy(wqkv_h.at[:, pl.ds(lo, n)], wq_raw.at[:, pl.ds(lo, n)], sems.at[k])

    cwa, cwb, cwc = wcopy(0, 512, 640), wcopy(1, 1152, 576), wcopy(7, 0, 512)
    co = pltpu.make_async_copy(wo_h, wo_raw, sems.at[2])
    c1 = pltpu.make_async_copy(w1_h, w1, sems.at[3])
    c2 = pltpu.make_async_copy(w2t_h, w2t, sems.at[4])
    cb1 = pltpu.make_async_copy(b1_h, b1v, sems.at[5])
    cb2 = pltpu.make_async_copy(b2_h, b2v, sems.at[6])

    def with_ones(v, j):
        w, u = WIN[j], ZROW[j]
        g = (u // 16) * 16
        sel = lax.broadcasted_iota(jnp.int32, (16, TS), 0) == (u - g)
        mid = jnp.where(sel, jnp.ones((16, TS), BF), v[w + g:w + g + 16])
        parts = ([v[w:w + g]] if g > 0 else []) + [mid] + ([v[w + g + 16:w + 128]] if g + 16 < 128 else [])
        return jnp.concatenate(parts, axis=0)

    def ln_stats(b, anch):
        r = D // len(anch)
        c = xs[b, 0:16, :].astype(F32)[0:1]
        s1 = s2 = None
        for g, a in enumerate(anch):
            t1, t2 = _part_sums(xs[b, g * r:(g + 1) * r, :].astype(F32) - (c + _dep_zero(a)[0:1]))
            s1, s2 = (t1, t2) if s1 is None else (s1 + t1, s2 + t2)
        return _ln_stats(s1, s2, c)

    def ln_store(b, slot, m, rstd, anch):
        r = D // len(anch)
        for g, a in enumerate(anch):
            lnb[slot, g * r:(g + 1) * r, :] = (
                (xs[b, g * r:(g + 1) * r, :].astype(F32) - (m + _dep_zero(a)[0:1])) * rstd).astype(BF)

    def kv_dots(pk, v, first):
        for j, w in enumerate(WIN):
            t = lax.dot_general(with_ones(v, j), pk[w:w + 128], NT, preferred_element_type=F32)
            kvacc[j] = t if first else kvacc[j] + t

    def proj(lo, c, ln):
        return jnp.dot(wqT[lo + c * RC:lo + (c + 1) * RC, :], ln, preferred_element_type=F32)

    def p1_block(i, nxt, nslot):
        ln = lnb[i]
        res = [proj(D, c, ln) for c in range(NR)]
        pk = _phi(jnp.concatenate(res, axis=0)).astype(BF)
        res += [proj(2 * D, c, ln) for c in range(NR)]
        v = jnp.concatenate(res[NR:], axis=0).astype(BF)
        m, rstd = ln_stats(nxt, [res[a][0:8] for a in (0, 1, 2, 3)])
        lq = lnb[i - G]
        res += [proj(0, c, lq) for c in range(NR)]
        kv_dots(pk, v, False)
        ln_store(nxt, nslot, m, rstd, [res[a][0:8] for a in (5, 6, 7, 8)])
        pqs[i - G] = _phi(jnp.concatenate(res[2 * NR:], axis=0)).astype(BF)

    def att_ps(i):
        pq = pqs[i]
        den = jnp.dot(zw[...], _wins(pq), preferred_element_type=F32)
        return pq.astype(F32) * _expand_heads(_recip(den + 1e-6))

    def att_dot(ps):
        psw = _wins(ps)
        return jnp.concatenate([jnp.dot(mT[c * RC:(c + 1) * RC, :], psw, preferred_element_type=F32)
                                for c in range(NR)], axis=0)

    def att_fin(i, slot, att):
        h = xs[i].astype(F32) + att
        hb[slot] = h
        c = h[0:1, :]
        m, rstd = _ln_stats(*_part_sums(h - c), c)
        ln2b[slot] = ((hb[slot] - m) * rstd).astype(BF).T

    def ffn1(ln2, c):
        a1 = jnp.dot(ln2, w1[:, c * CH:(c + 1) * CH], preferred_element_type=F32)
        r = jnp.maximum(a1 + b1r[0:1, c * CH:(c + 1) * CH], 0.0)
        return (r * r).astype(BF)

    def p2_block(i, slot):
        ln2 = ln2b[slot]
        ps = att_ps(i + 1).astype(BF)
        rs = [ffn1(ln2, c) for c in range(3)]
        att_fin(i + 1, 1 - slot, att_dot(ps))
        rs += [ffn1(ln2, c) for c in range(3, NC)]
        o = lax.dot_general(w2t[...], jnp.concatenate(rs, axis=1), NT, preferred_element_type=F32)
        obuf[i] = (o + (hb[slot] + b2c[:, 0:1])).astype(BF)
        ocopy(i).start()

    for c in (xcopy(0), cb1, cb2, cwa, xcopy(1), cwb, cwc, xcopy(2), co):
        c.start()
    for b in range(3, NB):
        xcopy(b).start()
    c1.start()
    c2.start()
    for j, w in enumerate(WIN):
        hr = _head_of(lax.broadcasted_iota(jnp.int32, (128, 128), 0) + w)
        hc = _head_of(lax.broadcasted_iota(jnp.int32, (128, 128), 1) + w)
        msks[j] = jnp.where((hr == hc) & (hr >= HLO[j]) & (hr < HHI[j]), 1.0, 0.0)
        hsel = lax.broadcasted_iota(jnp.int32, (32, 128), 0)
        hd = _head_of(lax.broadcasted_iota(jnp.int32, (32, 128), 1) + w)
        zmsk[:, 128 * j:128 * j + 128] = jnp.where((hd == hsel) & (hd >= HLO[j]) & (hd < HHI[j]), 1.0, 0.0)
    xcopy(0).wait()
    cb1.wait()
    cb2.wait()
    x0 = xs[0].astype(F32)
    c0 = x0[0:1, :]
    m, rstd = _ln_stats(*_part_sums(x0 - c0), c0)
    lnb[0] = ((x0 - m) * rstd).astype(BF)
    b2c[...] = jnp.broadcast_to(b2v[...].astype(F32).reshape(1, D), (128, D)).T
    b1r[...] = jnp.broadcast_to(b1v[...].astype(F32).reshape(1, F), (8, F))
    cwa.wait()
    wqT[512:1152, :] = wq_raw[:, 512:1152].T
    xcopy(1).wait()
    kk = [proj(D, c, lnb[0]) for c in range(NR)]
    m, rstd = ln_stats(1, [kk[0][0:8], kk[0][0:8], kk[1][0:8], kk[1][0:8]])
    kvacc[0, 0:8, :] = jnp.zeros((8, 128), F32)
    ln_store(1, 1, m, rstd, [kk[2][0:8], kk[2][0:8], kk[3][0:8], kk[3][0:8]])
    pk0 = _phi(jnp.concatenate(kk, axis=0)).astype(BF)
    cwb.wait()
    ln1 = lnb[1]
    pk1 = _phi(jnp.concatenate([proj(D, c, ln1) for c in range(NR)], axis=0)).astype(BF)
    wqT[1152:1728, :] = wq_raw[:, 1152:1728].T
    cwc.wait()
    xcopy(2).wait()
    vs = [jnp.concatenate([proj(2 * D, c, lnb[b]) for c in range(NR)], axis=0) for b in range(2)]
    wqT[0:512, :] = wq_raw[:, 0:512].T
    m, rstd = ln_stats(2, [vs[0][a * RC:a * RC + 8] for a in range(4)])
    kv_dots(pk0, vs[0].astype(BF), True)
    kv_dots(pk1, vs[1].astype(BF), False)
    ln_store(2, 2, m, rstd, [vs[1][a * RC:a * RC + 8] for a in range(4)])
    co.wait()

    ng = (NB - G) // G

    def p1(g, carry):
        b0 = G + g * G

        @pl.when(g + 1 < ng)
        def _():
            for u in range(1, G + 1):
                xcopy(b0 + u).wait()

        @pl.when(g + 1 == ng)
        def _():
            for u in range(1, G):
                xcopy(b0 + u).wait()

        for u in range(2):
            jw = jnp.minimum(2 * g + u, 4)
            woT[jw] = wo_raw[pl.ds(pl.multiple_of(jw * 112, 16), 128), :].T
        for u in range(G):
            p1_block(b0 + u, jnp.minimum(b0 + u + 1, NB - 1), b0 + u + 1)
        return carry

    lax.fori_loop(0, ng, p1, 0)

    c1.wait()
    c2.wait()
    qs = [[], []]
    filled = [0]

    def qn():
        u, c = divmod(filled[0], NR)
        qs[u].append(proj(0, c, lnb[NB - G + u]))
        filled[0] += 1
        if c == NR - 1:
            pqs[NB - G + u] = _phi(jnp.concatenate(qs[u], axis=0)).astype(BF)

    qn()
    for j in range(5):
        z = kvacc[j, ZROW[j]:ZROW[j] + 1, :]
        zw[:, 128 * j:128 * j + 128] = (zmsk[:, 128 * j:128 * j + 128] * jnp.broadcast_to(z, (32, 128))).astype(BF)
    ps0 = att_ps(0)
    qn()
    for j, a in enumerate((-1, -1, 0, 280, 568)):
        kvm = jnp.where(msks[j] > 0.5, kvacc[j], 0.0)
        if a >= 0:
            kvm = kvm + _dep_zero(ps0[a:a + 8])[0:1, 0:128]
        kvm = kvm.astype(BF)
        for c in range(NR):
            mT[c * RC:(c + 1) * RC, 128 * j:128 * j + 128] = jnp.dot(
                woT[j, c * RC:(c + 1) * RC, :], kvm, preferred_element_type=F32).astype(BF)
    qn()
    att0 = att_dot(ps0.astype(BF))
    for _ in range(2 * NR - 3):
        qn()
    att_fin(0, 0, att0)

    lax.fori_loop(0, NB - 1, lambda i, c: (p2_block(i, i % 2), c)[1], 0)

    i, slot = NB - 1, (NB - 1) % 2
    ln2 = ln2b[slot]
    r = jnp.concatenate([ffn1(ln2, c) for c in range(NC)], axis=1)
    last = []
    for u in range(TS // 128):
        nr = 1 if u + 1 < TS // 128 else 4
        rr = D // nr
        for c in range(nr):
            rows, cols = slice(c * rr, (c + 1) * rr), slice(128 * u, 128 * u + 128)
            o = lax.dot_general(w2t[rows, :], r[cols], NT, preferred_element_type=F32)
            obuf[i, rows, cols] = (o + (hb[slot, rows, cols] + b2c[rows, 0:1])).astype(BF)
            cp = pltpu.make_async_copy(obuf.at[i, pl.ds(c * rr, rr), pl.ds(128 * u, 128)],
                                       o_h.at[pl.ds(c * rr, rr), pl.ds(i * TS + 128 * u, 128)],
                                       esems.at[len(last)])
            cp.start()
            last.append(cp)
    for b in range(NB - 1):
        ocopy(b).wait()
    for cp in last:
        cp.wait()


@jax.jit
def pallas_sequential_preLN__linear_attn_block__dense_activation_squared_relu__prompt_kernel(
    A_x: jax.Array,
    A_wqkv: jax.Array,
    A_wo: jax.Array,
    B_x: jax.Array,
    B_w1: jax.Array,
    B_b1: jax.Array,
    B_w2: jax.Array,
    B_b2: jax.Array,
):
    del B_x
    hbm = pl.BlockSpec(memory_space=pl.ANY)
    vmem = pltpu.VMEM
    out_t = pl.pallas_call(
        _kernel,
        out_shape=jax.ShapeDtypeStruct((D, S), BF),
        in_specs=[hbm] * 7,
        out_specs=hbm,
        scratch_shapes=[
            vmem((NB, D, TS), BF),
            vmem((D, 3 * D), BF),
            vmem((3 * D, D), BF),
            vmem((D, D), BF),
            vmem((5, D, 128), BF),
            vmem((D, F), BF),
            vmem((D, F), BF),
            vmem((F,), BF),
            vmem((D,), BF),
            vmem((NB + 1, D, TS), BF),
            vmem((NB, D, TS), BF),
            vmem((5, 128, 128), F32),
            vmem((D, 640), BF),
            vmem((32, 640), BF),
            vmem((5, 128, 128), F32),
            vmem((32, 640), F32),
            vmem((D, 128), F32),
            vmem((8, F), F32),
            vmem((2, TS, D), BF),
            vmem((2, D, TS), F32),
            vmem((NB, D, TS), BF),
            pltpu.SemaphoreType.DMA((8 + NB,)),
            pltpu.SemaphoreType.DMA((NB - 1,)),
            pltpu.SemaphoreType.DMA((5,)),
        ],
        compiler_params=pltpu.CompilerParams(vmem_limit_bytes=110 * 2**20),
    )(A_x[0].T, A_wqkv, A_wo, B_w1, B_b1, B_w2.T, B_b2)
    return out_t.T[None]
```
